```python
import os as _os
_os.environ.setdefault('JAX_PLATFORMS', 'cpu')
import jax
import jax.numpy as jnp

def _softmax(x, axis=-1):
    return jax.nn.softmax(x, axis=axis)

def _gelu(x):
    return jax.nn.gelu(x, approximate=True)

def _silu(x):
    return jax.nn.silu(x)

def _sigmoid(x):
    return jax.nn.sigmoid(x)

def _layernorm(x, axis=-1, eps=1e-05):
    m = jnp.mean(x, axis=axis, keepdims=True)
    v = jnp.var(x, axis=axis, keepdims=True)
    return (x - m) / jnp.sqrt(v + eps)

def _scatter_add(tgt, idx, src, axis=0):
    return tgt.at[idx].add(src)

def _segment_sum(src, seg, n):
    return jax.ops.segment_sum(src, seg, n)

class _Rng:

    def __init__(self, key):
        self._k = key

    def _next(self):
        self._k, sub = jax.random.split(self._k)
        return sub

    def normal(self, shape):
        return jax.random.normal(self._next(), shape, dtype=jnp.bfloat16)

    def randint(self, lo, hi, shape):
        return jax.random.randint(self._next(), shape, lo, hi, dtype=jnp.int32)

    def uniform(self, shape, lo=0.0, hi=1.0):
        return jax.random.uniform(self._next(), shape, jnp.bfloat16, lo, hi)

    def permutation(self, n):
        return jax.random.permutation(self._next(), n)
kernel_name = 'parallel_sum__memory_aug_recurrent_mem_tr__dense_activation_gelu__prompt'

def setup_inputs():
    _rng = _Rng(jax.random.key(int.from_bytes(__import__("os").urandom(4), "little")))
    _w = lambda a: (lambda t: t.astype(jnp.bfloat16) if jnp.issubdtype(t.dtype, jnp.floating) else t)(jnp.asarray(a))

    def _A_setup():
        B, S, Dm = (1, 2048, 1024)
        H, Dh = (32, 128)
        M, seg = (8, 32)
        seg = min(seg, S)
        S = S // seg * seg
        return {'x': _w((lambda *s: _rng.normal(s) * 0.05)(B, S, Dm)), 'mem0': _w((lambda *s: _rng.normal(s) * 0.2)(B, M, Dm)), 'Wq': _w((lambda *s: _rng.normal(s) * 0.8)(Dm, H, Dh) * Dm ** (-0.5)), 'Wk': _w((lambda *s: _rng.normal(s) * 0.8)(Dm, H, Dh) * Dm ** (-0.5)), 'Wv': _w((lambda *s: _rng.normal(s) * 0.2)(Dm, H, Dh) * Dm ** (-0.5)), 'Wo': _w((lambda *s: _rng.normal(s) * 0.2)(H, Dh, Dm) * (H * Dh) ** (-0.5)), 'seg_len': seg}
    _A_in = _A_setup()

    def _B_setup():
        B, S, D, F = (1, 2048, 1024, 3584)
        return {'x': _w((lambda *s: _rng.normal(s) * 0.05)(B, S, D)), 'w1': _w((lambda *s: _rng.normal(s) * 0.1)(D, F) * D ** (-0.5)), 'b1': _w((lambda *s: _rng.normal(s) * 0.1)(F) * 0.01), 'w2': _w((lambda *s: _rng.normal(s) * 0.1)(F, D) * F ** (-0.5)), 'b2': _w((lambda *s: _rng.normal(s) * 0.05)(D) * 0.01)}
    _B_in = _B_setup()
    return {'A_x': _A_in['x'], 'A_mem0': _A_in['mem0'], 'A_Wq': _A_in['Wq'], 'A_Wk': _A_in['Wk'], 'A_Wv': _A_in['Wv'], 'A_Wo': _A_in['Wo'], 'A_seg_len': _A_in['seg_len'], 'B_x': _B_in['x'], 'B_w1': _B_in['w1'], 'B_b1': _B_in['b1'], 'B_w2': _B_in['w2'], 'B_b2': _B_in['b2']}

def reference(A_x, A_mem0, A_Wq, A_Wk, A_Wv, A_Wo, A_seg_len, B_x, B_w1, B_b1, B_w2, B_b2):

    def _A_ref(x, mem0, Wq, Wk, Wv, Wo, seg_len):
        B, S, Dm = x.shape
        H, Dh = (Wq.shape[1], Wq.shape[2])
        M = mem0.shape[1]
        scale = Dh ** (-0.5)
        n_seg = S // seg_len
        L = M + seg_len
        idx = jnp.arange(L)
        mask = (idx[:, None] < M) | (idx[:, None] >= idx[None, :])
        mem = mem0
        outs = []
        for s in range(n_seg):
            xs = x[:, s * seg_len:(s + 1) * seg_len, :].copy()
            h = jnp.concatenate([mem, xs], axis=1)
            q = jnp.einsum('btd,dhe->bhte', h, Wq)
            k = jnp.einsum('btd,dhe->bhte', h, Wk)
            v = jnp.einsum('btd,dhe->bhte', h, Wv)
            scores = jnp.einsum('bhqe,bhke->bhqk', q, k) * scale
            scores = jnp.where(mask[None, None], scores, -1000000000.0)
            p = _softmax(scores, axis=-1)
            o = jnp.einsum('bhqk,bhke->bhqe', p, v)
            o = jnp.einsum('bhte,hed->btd', o, Wo)
            mem = o[:, :M, :].copy()
            outs.append(o[:, M:, :])
        return jnp.concatenate(outs, axis=1)

    def _B_ref(x, w1, b1, w2, b2):
        h = jnp.einsum('bsd,df->bsf', x, w1) + b1
        h = _gelu(h)
        return jnp.einsum('bsf,fd->bsd', h, w2) + b2
    x = A_x
    xn = _layernorm(x, axis=-1)
    return x + _A_ref(xn, A_mem0, A_Wq, A_Wk, A_Wv, A_Wo, A_seg_len) + _B_ref(xn, B_w1, B_b1, B_w2, B_b2)
```

```python
import functools

import jax
import jax.numpy as jnp
from jax import lax
import jax.experimental.pallas as pl
import jax.experimental.pallas.tpu as pltpu

S, D, H, DH, M, SEG, F = 2048, 1024, 32, 128, 8, 32, 3584
L = M + SEG
NSEG = S // SEG
FC = 512
NFC = F // FC
RB = 1024
NRB = S // RB
NSUB = 8
SB = RB // NSUB
LB = 256
NEG = -1e9
BT, FT = 5, 11
UNR = 4
WOFF = 512
CW = 2
NIT = (NFC - CW) * NRB
UPI = (48 + NIT - 1) // NIT
IT0 = CW * NRB
NPART = 4 * NSUB
H1 = 28


def _dot(a, b):
    return lax.dot_general(a, b, (((1,), (0,)), ((), ())), preferred_element_type=jnp.float32)


def _dot_nt(a, b):
    return lax.dot_general(a, b, (((1,), (1,)), ((), ())), preferred_element_type=jnp.float32)


def _kernel(x_hbm, mem0_ref, wq_hbm, wk_hbm, wv_hbm, wo_hbm, w1_hbm, b1_ref, w2_hbm, b2_ref,
            o_hbm,
            x_s, xn_s, res_s, w1_s, w2_s, big_s, stage_s, wo_s,
            sem_x, sem_w1, sem_w2, sem_st, sem_wo, sem_o):
    def x_copy(r):
        r0 = pl.multiple_of(r * LB, LB)
        return pltpu.make_async_copy(x_hbm.at[pl.ds(r0, LB), :], x_s.at[pl.ds(r0, LB), :], sem_x.at[r])

    def w1_copy(c):
        c0 = pl.multiple_of(c * FC, FC)
        return pltpu.make_async_copy(w1_hbm.at[:, pl.ds(c0, FC)], w1_s.at[c], sem_w1.at[c])

    def w2_copy(c):
        c0 = pl.multiple_of(c * FC, FC)
        return pltpu.make_async_copy(w2_hbm.at[pl.ds(c0, FC), :], w2_s.at[c], sem_w2.at[c])

    def issue_x(r, carry):
        x_copy(r).start()
        return carry
    lax.fori_loop(0, S // LB, issue_x, 0)

    def issue_w(c, carry):
        w1_copy(c).start()
        w2_copy(c).start()
        return carry
    lax.fori_loop(0, NFC, issue_w, 0)

    c_st = [pltpu.make_async_copy(w.bitcast(jnp.uint32).at[:, i, :], stage_s.at[m * 32 + i], sem_st.at[m])
            for m, w in enumerate((wq_hbm, wk_hbm, wv_hbm)) for i in range(32)]
    c_wo = [pltpu.make_async_copy(wo_hbm.bitcast(jnp.uint32).at[:, pl.ds(n * 128, 128)], wo_s.at[n], sem_wo.at[0])
            for n in range(8)]
    late_copies = c_st + c_wo

    b1f = pltpu.bitcast(b1_ref[...].astype(jnp.float32), jnp.uint32)
    for i in range(F // 128):
        big_s[i * 8:(i + 1) * 8, :] = jnp.broadcast_to(b1f[i:i + 1, :], (8, 128))
    b2f = b2_ref[...].astype(jnp.float32)
    b2row = jnp.concatenate([b2f[n:n + 1, :] for n in range(D // 128)], axis=1)

    def ln_body(r, carry):
        x_copy(r).wait()
        r0 = pl.multiple_of(r * LB, LB)
        xb = x_s[pl.ds(r0, LB), :].astype(jnp.float32)
        mu = jnp.mean(xb, axis=-1, keepdims=True)
        xc = xb - mu
        var = jnp.mean(xc * xc, axis=-1, keepdims=True)
        xn = xc * lax.rsqrt(var + 1e-5)
        xn_s[pl.ds(r0, LB), :] = xn.astype(jnp.bfloat16)
        res_s[pl.ds(r0, LB), :] = xb + b2row
        return carry
    lax.fori_loop(0, S // LB, ln_body, 0)

    def rp_part(p, it):
        tot = UPI * 64
        lo_, hi_ = (tot * p) // NPART, (tot * (p + 1)) // NPART
        for k in range(UPI):
            a0, a1 = max(lo_, k * 64) - k * 64, min(hi_, (k + 1) * 64) - k * 64
            if a1 <= a0:
                continue
            unit = (it - IT0) * UPI + k
            valid = jnp.logical_and(it >= IT0, unit < 48)
            m = unit // 16
            hp = unit % 16
            ei = jnp.where(valid, m * 32 + hp, 96)
            oi = jnp.where(valid, m * 32 + 16 + hp, 97)
            di = jnp.where(valid, m * 32 + 2 * hp, 96)
            e = stage_s[ei, a0 * 8:a1 * 8, :]
            o = stage_s[oi, a0 * 8:a1 * 8, :]
            lo = (e & jnp.uint32(0xFFFF)) | (o << 16)
            hi = (e >> 16) | (o & jnp.uint32(0xFFFF0000))
            d0 = pl.multiple_of(WOFF + di * 512 + a0 * 8, 8)
            big_s[pl.ds(d0, (a1 - a0) * 8), :] = lo
            big_s[pl.ds(d0 + 512, (a1 - a0) * 8), :] = hi

    def ffn_chunk(c, carry):
        w1_copy(c).wait()
        w2_copy(c).wait()
        for k in range(4):
            @pl.when(c == k)
            def _():
                for cp in late_copies[k * 32:(k + 1) * 32]:
                    cp.start()
        for m_ in range(3):
            first_it = IT0 + (16 * m_) // UPI
            assert first_it // NRB > m_

            @pl.when(c == first_it // NRB)
            def _():
                for cp in c_st[m_ * 32:(m_ + 1) * 32]:
                    cp.wait()

        def ffn_body(r, carry2):
            hc = {}

            def up(u):
                r0 = pl.multiple_of(r * RB + u * SB, SB)
                xb = xn_s[pl.ds(r0, SB), :]
                hs = []
                for i in range(FC // 128):
                    rp_part(u * 4 + i, c * NRB + r)
                    b0 = pl.multiple_of((c * 4 + i) * 8, 8)
                    b8 = pltpu.bitcast(big_s[pl.ds(b0, 8), :], jnp.float32)
                    a = _dot(xb, w1_s[c, :, i * 128:(i + 1) * 128]) + jnp.tile(b8, (SB // 8, 1))
                    g = jax.nn.gelu(a, approximate=True)
                    hs.append(g.astype(jnp.bfloat16))
                hc[u] = jnp.concatenate(hs, axis=1)

            def down(u):
                r0 = pl.multiple_of(r * RB + u * SB, SB)
                hcat = hc.pop(u)
                for n in range(D // 128):
                    y = _dot(hcat, w2_s[c, :, n * 128:(n + 1) * 128])
                    res_s[pl.ds(r0, SB), n * 128:(n + 1) * 128] += y

            up(0)
            for u in range(NSUB):
                if u + 1 < NSUB:
                    up(u + 1)
                down(u)
            return carry2
        lax.fori_loop(0, NRB, ffn_body, 0)
        return carry
    lax.fori_loop(0, NFC, ffn_chunk, 0)
    for cp in c_wo:
        cp.wait()

    ri = lax.broadcasted_iota(jnp.int32, (L, 128), 0)
    ci = lax.broadcasted_iota(jnp.int32, (L, 128), 1)
    mask = ((ri < M) | (ri >= ci)) & (ci < L)
    scale = DH ** (-0.5)
    zpad = jnp.zeros((128 - L, DH), jnp.float32)

    def wrows(idx, a, b):
        return pltpu.bitcast(big_s[WOFF + idx * 512 + a:WOFF + idx * 512 + b, :], jnp.bfloat16)

    def out_copy(s):
        r0 = pl.multiple_of(s * SEG, SEG)
        return pltpu.make_async_copy(x_s.at[pl.ds(r0, SEG), :], o_hbm.at[pl.ds(r0, SEG), :], sem_o.at[0])

    def step(s, mem, maybe_first):
        if maybe_first:
            @pl.when(s > 0)
            def _():
                out_copy(s - 1).start()
        else:
            out_copy(s - 1).start()
        r0 = pl.multiple_of(s * SEG, SEG)
        xs = xn_s[pl.ds(r0, SEG), :].astype(jnp.float32)
        h = jnp.concatenate([mem, xs], axis=0)
        q_, k_, v_, p_, o_ = {}, {}, {}, {}, {}
        pre = {idx: _dot(h[:, :512], wrows(idx, 0, 256)) for idx in (0, 32, 64)}

        def proj(idx):
            if idx in pre:
                return _dot(h[:, 512:], wrows(idx, 256, 512)) + pre.pop(idx)
            return _dot(h, wrows(idx, 0, 512))

        def padded(t):
            return jnp.concatenate([t, zpad], axis=0).astype(jnp.bfloat16)

        def scores(j):
            sc = _dot_nt(q_.pop(j), k_.pop(j))
            t = jnp.where(mask, sc * scale, NEG)
            m = jnp.max(t, axis=1, keepdims=True)
            e = jnp.exp(t - m)
            l = jnp.sum(e, axis=1, keepdims=True)
            r_ = pl.reciprocal(l, approx=True)
            p_[j] = e * (r_ * (2.0 - l * r_))

        def values(j):
            o_[j] = _dot(p_.pop(j), v_.pop(j))

        def emit(t):
            if (t - BT) % 3 == 0 and 0 <= (t - BT) // 3 < H:
                scores((t - BT) // 3)
            if (t - FT) % 3 == 0 and 0 <= (t - FT) // 3 < H:
                values((t - FT) // 3)

        for i in range(H):
            q_[i] = proj(i)
            emit(3 * i)
            k_[i] = padded(proj(32 + i))
            emit(3 * i + 1)
            v_[i] = padded(proj(64 + i))
            emit(3 * i + 2)

        tail = sorted([(3 * j + BT, 0, j) for j in range(H) if 3 * j + BT >= 3 * H] +
                      [(3 * j + FT, 1, j) for j in range(H) if 3 * j + FT >= 3 * H])
        assert all(j >= H1 for _, _, j in tail)
        part1 = []

        def wo_part1(n):
            o1 = jnp.concatenate([o_[j] for j in range(H1)], axis=1)
            part1.append(_dot(o1, pltpu.bitcast(wo_s[n, 0:H1 * 64, :], jnp.bfloat16)))

        wo_part1(0)
        n_done = 1
        clock = 3 * H - 1 + 3.5
        for t, kind, j in tail:
            while clock < t and n_done < 8:
                wo_part1(n_done)
                n_done += 1
                clock += 3.5
            (scores if kind == 0 else values)(j)
        while n_done < 8:
            wo_part1(n_done)
            n_done += 1
        o2 = jnp.concatenate([o_[j] for j in range(H1, H)], axis=1)
        outs = [_dot(o2, pltpu.bitcast(wo_s[n, H1 * 64:H * 64, :], jnp.bfloat16)) + part1[n] for n in range(8)]
        out = jnp.concatenate(outs, axis=1)
        fin = res_s[pl.ds(r0, SEG), :] + out[M:]
        x_s[pl.ds(r0, SEG), :] = fin.astype(jnp.bfloat16)
        return out[:M].astype(jnp.bfloat16).astype(jnp.float32)

    def steps(i, mem):
        for u in range(UNR):
            mem = step(i * UNR + u, mem, u == 0)
        return mem
    lax.fori_loop(0, NSEG // UNR, steps, mem0_ref[...].astype(jnp.float32))
    out_copy(NSEG - 1).start()
    pltpu.make_async_copy(x_s, o_hbm, sem_o.at[0]).wait()


@functools.partial(jax.jit, static_argnames=("A_seg_len",))
def pallas_parallel_sum__memory_aug_recurrent_mem_tr__dense_activation_gelu__prompt_kernel(
    A_x: jax.Array,
    A_mem0: jax.Array,
    A_Wq: jax.Array,
    A_Wk: jax.Array,
    A_Wv: jax.Array,
    A_Wo: jax.Array,
    A_seg_len: int,
    B_x: jax.Array,
    B_w1: jax.Array,
    B_b1: jax.Array,
    B_w2: jax.Array,
    B_b2: jax.Array,
):
    del B_x
    assert A_x.shape == (1, S, D) and A_mem0.shape == (1, M, D) and int(A_seg_len) == SEG
    assert A_Wq.shape == (D, H, DH) and A_Wo.shape == (H, DH, D) and B_w1.shape == (D, F)
    x = A_x.reshape(S, D)
    mem0 = A_mem0.reshape(M, D)
    wq = A_Wq.reshape(D // 2, 2 * H, DH)
    wk = A_Wk.reshape(D // 2, 2 * H, DH)
    wv = A_Wv.reshape(D // 2, 2 * H, DH)
    wo = A_Wo.reshape(H * DH, D)
    b1 = B_b1.reshape(F // 128, 128)
    b2 = B_b2.reshape(D // 128, 128)
    any_spec = pl.BlockSpec(memory_space=pl.ANY)
    vm = pl.BlockSpec(memory_space=pltpu.VMEM)
    out = pl.pallas_call(
        _kernel,
        out_shape=jax.ShapeDtypeStruct((S, D), jnp.bfloat16),
        in_specs=[any_spec, vm, any_spec, any_spec, any_spec, any_spec, any_spec, vm, any_spec, vm],
        out_specs=any_spec,
        scratch_shapes=[
            pltpu.VMEM((S, D), jnp.bfloat16),
            pltpu.VMEM((S, D), jnp.bfloat16),
            pltpu.VMEM((S, D), jnp.float32),
            pltpu.VMEM((NFC, D, FC), jnp.bfloat16),
            pltpu.VMEM((NFC, FC, D), jnp.bfloat16),
            pltpu.VMEM((WOFF + 98 * 512, 128), jnp.uint32),
            pltpu.VMEM((98, D // 2, DH), jnp.uint32),
            pltpu.VMEM((8, H * DH // 2, 128), jnp.uint32),
            pltpu.SemaphoreType.DMA((S // LB,)),
            pltpu.SemaphoreType.DMA((NFC,)),
            pltpu.SemaphoreType.DMA((NFC,)),
            pltpu.SemaphoreType.DMA((3,)),
            pltpu.SemaphoreType.DMA((1,)),
            pltpu.SemaphoreType.DMA((1,)),
        ],
        compiler_params=pltpu.CompilerParams(vmem_limit_bytes=120 * 1024 * 1024),
    )(x, mem0, wq, wk, wv, wo, B_w1, b1, B_w2, b2)
    return out.reshape(1, S, D)
```

```python
import functools

import jax
import jax.numpy as jnp
from jax import lax
import jax.experimental.pallas as pl
import jax.experimental.pallas.tpu as pltpu

S, D, H, DH, M, SEG, F = 2048, 1024, 32, 128, 8, 32, 3584
L = M + SEG
NSEG = S // SEG
FC = 512
NFC = F // FC
RB = 1024
NRB = S // RB
NSUB = 8
SB = RB // NSUB
LB = 256
NEG = -1e9
BT, FT = 5, 11
UNR = 4
B2OFF = 256
WOFF = 512
CW = 2
NIT = (NFC - CW) * NRB
UPI = (48 + NIT - 1) // NIT
IT0 = CW * NRB
NPART = 4 * NSUB
H1 = 28


def _dot(a, b):
    return lax.dot_general(a, b, (((1,), (0,)), ((), ())), preferred_element_type=jnp.float32)


def _dot_nt(a, b):
    return lax.dot_general(a, b, (((1,), (1,)), ((), ())), preferred_element_type=jnp.float32)


def _kernel(x_hbm, mem0_ref, wq_hbm, wk_hbm, wv_hbm, wo_hbm, w1_hbm, b1_ref, w2_hbm, b2_ref,
            o_hbm,
            x_s, xn_s, res_s, w1_s, w2_s, big_s, stage_s, wo_s,
            sem_x, sem_w1, sem_w2, sem_st, sem_wo, sem_o):
    def x_copy(r):
        r0 = pl.multiple_of(r * LB, LB)
        return pltpu.make_async_copy(x_hbm.at[pl.ds(r0, LB), :], x_s.at[pl.ds(r0, LB), :], sem_x.at[r])

    def w1_copy(c):
        c0 = pl.multiple_of(c * FC, FC)
        return pltpu.make_async_copy(w1_hbm.at[:, pl.ds(c0, FC)], w1_s.at[c], sem_w1.at[c])

    def w2_copy(c):
        c0 = pl.multiple_of(c * FC, FC)
        return pltpu.make_async_copy(w2_hbm.at[pl.ds(c0, FC), :], w2_s.at[c], sem_w2.at[c])

    def issue_x(lo, hi):
        def body(r, carry):
            x_copy(r).start()
            return carry
        lax.fori_loop(lo, hi, body, 0)

    def issue_w(lo, hi):
        def body(c, carry):
            w1_copy(c).start()
            w2_copy(c).start()
            return carry
        lax.fori_loop(lo, hi, body, 0)

    issue_x(0, RB // LB)
    issue_w(0, 1)
    issue_x(RB // LB, S // LB)
    issue_w(1, NFC)

    c_st = [pltpu.make_async_copy(w.bitcast(jnp.uint32).at[:, i, :], stage_s.at[m * 32 + i], sem_st.at[m])
            for m, w in enumerate((wq_hbm, wk_hbm, wv_hbm)) for i in range(32)]
    c_wo = [pltpu.make_async_copy(wo_hbm.bitcast(jnp.uint32).at[:, pl.ds(n * 128, 128)], wo_s.at[n], sem_wo.at[0])
            for n in range(8)]
    late_copies = c_st + c_wo

    b1f = pltpu.bitcast(b1_ref[...].astype(jnp.float32), jnp.uint32)
    for i in range(F // 128):
        big_s[i * 8:(i + 1) * 8, :] = jnp.broadcast_to(b1f[i:i + 1, :], (8, 128))
    b2f = pltpu.bitcast(b2_ref[...].astype(jnp.float32), jnp.uint32)
    for n in range(D // 128):
        big_s[B2OFF + n * 8:B2OFF + (n + 1) * 8, :] = jnp.broadcast_to(b2f[n:n + 1, :], (8, 128))

    def ln_body(r, carry):
        x_copy(r).wait()
        r0 = pl.multiple_of(r * LB, LB)
        xb = x_s[pl.ds(r0, LB), :].astype(jnp.float32)
        mu = jnp.mean(xb, axis=-1, keepdims=True)
        xc = xb - mu
        var = jnp.mean(xc * xc, axis=-1, keepdims=True)
        xn = xc * lax.rsqrt(var + 1e-5)
        xn_s[pl.ds(r0, LB), :] = xn.astype(jnp.bfloat16)
        return carry

    def rp_part(p, it):
        tot = UPI * 64
        lo_, hi_ = (tot * p) // NPART, (tot * (p + 1)) // NPART
        for k in range(UPI):
            a0, a1 = max(lo_, k * 64) - k * 64, min(hi_, (k + 1) * 64) - k * 64
            if a1 <= a0:
                continue
            unit = (it - IT0) * UPI + k
            valid = jnp.logical_and(it >= IT0, unit < 48)
            m = unit // 16
            hp = unit % 16
            ei = jnp.where(valid, m * 32 + hp, 96)
            oi = jnp.where(valid, m * 32 + 16 + hp, 97)
            di = jnp.where(valid, m * 32 + 2 * hp, 96)
            e = stage_s[ei, a0 * 8:a1 * 8, :]
            o = stage_s[oi, a0 * 8:a1 * 8, :]
            lo = (e & jnp.uint32(0xFFFF)) | (o << 16)
            hi = (e >> 16) | (o & jnp.uint32(0xFFFF0000))
            d0 = pl.multiple_of(WOFF + di * 512 + a0 * 8, 8)
            big_s[pl.ds(d0, (a1 - a0) * 8), :] = lo
            big_s[pl.ds(d0 + 512, (a1 - a0) * 8), :] = hi

    def ffn_chunk(c, carry):
        for k in range(4):
            @pl.when(c == k)
            def _():
                for cp in late_copies[k * 32:(k + 1) * 32]:
                    cp.start()
        for m_ in range(3):
            first_it = IT0 + (16 * m_) // UPI
            assert first_it // NRB > m_

            @pl.when(c == first_it // NRB)
            def _():
                for cp in c_st[m_ * 32:(m_ + 1) * 32]:
                    cp.wait()

        def ffn_body(r, carry2):
            @pl.when(c == 0)
            def _():
                lax.fori_loop(r * (RB // LB), (r + 1) * (RB // LB), ln_body, 0)

            @pl.when(r == 0)
            def _():
                w1_copy(c).wait()
                w2_copy(c).wait()
            hc = {}

            def up(u):
                r0 = pl.multiple_of(r * RB + u * SB, SB)
                xb = xn_s[pl.ds(r0, SB), :]
                hs = []
                for i in range(FC // 128):
                    rp_part(u * 4 + i, c * NRB + r)
                    b0 = pl.multiple_of((c * 4 + i) * 8, 8)
                    b8 = pltpu.bitcast(big_s[pl.ds(b0, 8), :], jnp.float32)
                    a = _dot(xb, w1_s[c, :, i * 128:(i + 1) * 128]) + jnp.tile(b8, (SB // 8, 1))
                    g = jax.nn.gelu(a, approximate=True)
                    hs.append(g.astype(jnp.bfloat16))
                hc[u] = jnp.concatenate(hs, axis=1)

            def down(u):
                r0 = pl.multiple_of(r * RB + u * SB, SB)
                hcat = hc.pop(u)
                for n in range(D // 128):
                    y = _dot(hcat, w2_s[c, :, n * 128:(n + 1) * 128])
                    b8 = pltpu.bitcast(big_s[B2OFF + n * 8:B2OFF + (n + 1) * 8, :], jnp.float32)
                    prev = jnp.where(c == 0, jnp.tile(b8, (SB // 8, 1)),
                                     res_s[pl.ds(r0, SB), n * 128:(n + 1) * 128])
                    res_s[pl.ds(r0, SB), n * 128:(n + 1) * 128] = prev + y

            up(0)
            for u in range(NSUB):
                if u + 1 < NSUB:
                    up(u + 1)
                down(u)
            return carry2
        lax.fori_loop(0, NRB, ffn_body, 0)
        return carry
    lax.fori_loop(0, NFC, ffn_chunk, 0)
    for cp in c_wo:
        cp.wait()

    ri = lax.broadcasted_iota(jnp.int32, (L, 128), 0)
    ci = lax.broadcasted_iota(jnp.int32, (L, 128), 1)
    mask = ((ri < M) | (ri >= ci)) & (ci < L)
    scale = DH ** (-0.5)
    zpad = jnp.zeros((128 - L, DH), jnp.float32)

    def wrows(idx, a, b):
        return pltpu.bitcast(big_s[WOFF + idx * 512 + a:WOFF + idx * 512 + b, :], jnp.bfloat16)

    def out_copy(s):
        r0 = pl.multiple_of(s * SEG, SEG)
        return pltpu.make_async_copy(x_s.at[pl.ds(r0, SEG), :], o_hbm.at[pl.ds(r0, SEG), :], sem_o.at[0])

    def step(s, mem, maybe_first):
        if maybe_first:
            @pl.when(s > 0)
            def _():
                out_copy(s - 1).start()
        else:
            out_copy(s - 1).start()
        r0 = pl.multiple_of(s * SEG, SEG)
        xs = xn_s[pl.ds(r0, SEG), :].astype(jnp.float32)
        h = jnp.concatenate([mem, xs], axis=0)
        q_, k_, v_, p_, o_ = {}, {}, {}, {}, {}
        pre = {idx: _dot(h[:, :512], wrows(idx, 0, 256)) for idx in (0, 32, 64)}

        def proj(idx):
            if idx in pre:
                return _dot(h[:, 512:], wrows(idx, 256, 512)) + pre.pop(idx)
            return _dot(h, wrows(idx, 0, 512))

        def padded(t):
            return jnp.concatenate([t, zpad], axis=0).astype(jnp.bfloat16)

        def scores(j):
            sc = _dot_nt(q_.pop(j), k_.pop(j))
            t = jnp.where(mask, sc * scale, NEG)
            m = jnp.max(t, axis=1, keepdims=True)
            e = jnp.exp(t - m)
            l = jnp.sum(e, axis=1, keepdims=True)
            r_ = pl.reciprocal(l, approx=True)
            p_[j] = e * (r_ * (2.0 - l * r_))

        def values(j):
            o_[j] = _dot(p_.pop(j), v_.pop(j))

        def emit(t):
            if (t - BT) % 3 == 0 and 0 <= (t - BT) // 3 < H:
                scores((t - BT) // 3)
            if (t - FT) % 3 == 0 and 0 <= (t - FT) // 3 < H:
                values((t - FT) // 3)

        for i in range(H):
            q_[i] = proj(i)
            emit(3 * i)
            k_[i] = padded(proj(32 + i))
            emit(3 * i + 1)
            v_[i] = padded(proj(64 + i))
            emit(3 * i + 2)

        tail = sorted([(3 * j + BT, 0, j) for j in range(H) if 3 * j + BT >= 3 * H] +
                      [(3 * j + FT, 1, j) for j in range(H) if 3 * j + FT >= 3 * H])
        assert all(j >= H1 for _, _, j in tail)
        part1 = []

        def wo_part1(n):
            o1 = jnp.concatenate([o_[j] for j in range(H1)], axis=1)
            part1.append(_dot(o1, pltpu.bitcast(wo_s[n, 0:H1 * 64, :], jnp.bfloat16)))

        wo_part1(0)
        n_done = 1
        clock = 3 * H - 1 + 3.5
        for t, kind, j in tail:
            while clock < t and n_done < 8:
                wo_part1(n_done)
                n_done += 1
                clock += 3.5
            (scores if kind == 0 else values)(j)
        while n_done < 8:
            wo_part1(n_done)
            n_done += 1
        o2 = jnp.concatenate([o_[j] for j in range(H1, H)], axis=1)
        outs = [_dot(o2, pltpu.bitcast(wo_s[n, H1 * 64:H * 64, :], jnp.bfloat16)) + part1[n] for n in range(8)]
        out = jnp.concatenate(outs, axis=1)
        fin = (res_s[pl.ds(r0, SEG), :] + out[M:]) + x_s[pl.ds(r0, SEG), :].astype(jnp.float32)
        x_s[pl.ds(r0, SEG), :] = fin.astype(jnp.bfloat16)
        return out[:M]

    def steps(i, mem):
        for u in range(UNR):
            mem = step(i * UNR + u, mem, u == 0)
        return mem
    lax.fori_loop(0, NSEG // UNR, steps, mem0_ref[...].astype(jnp.float32))
    out_copy(NSEG - 1).start()
    pltpu.make_async_copy(x_s, o_hbm, sem_o.at[0]).wait()


@functools.partial(jax.jit, static_argnames=("A_seg_len",))
def pallas_parallel_sum__memory_aug_recurrent_mem_tr__dense_activation_gelu__prompt_kernel(
    A_x: jax.Array,
    A_mem0: jax.Array,
    A_Wq: jax.Array,
    A_Wk: jax.Array,
    A_Wv: jax.Array,
    A_Wo: jax.Array,
    A_seg_len: int,
    B_x: jax.Array,
    B_w1: jax.Array,
    B_b1: jax.Array,
    B_w2: jax.Array,
    B_b2: jax.Array,
):
    del B_x
    assert A_x.shape == (1, S, D) and A_mem0.shape == (1, M, D) and int(A_seg_len) == SEG
    assert A_Wq.shape == (D, H, DH) and A_Wo.shape == (H, DH, D) and B_w1.shape == (D, F)
    x = A_x.reshape(S, D)
    mem0 = A_mem0.reshape(M, D)
    wq = A_Wq.reshape(D // 2, 2 * H, DH)
    wk = A_Wk.reshape(D // 2, 2 * H, DH)
    wv = A_Wv.reshape(D // 2, 2 * H, DH)
    wo = A_Wo.reshape(H * DH, D)
    b1 = B_b1.reshape(F // 128, 128)
    b2 = B_b2.reshape(D // 128, 128)
    any_spec = pl.BlockSpec(memory_space=pl.ANY)
    vm = pl.BlockSpec(memory_space=pltpu.VMEM)
    out = pl.pallas_call(
        _kernel,
        out_shape=jax.ShapeDtypeStruct((S, D), jnp.bfloat16),
        in_specs=[any_spec, vm, any_spec, any_spec, any_spec, any_spec, any_spec, vm, any_spec, vm],
        out_specs=any_spec,
        scratch_shapes=[
            pltpu.VMEM((S, D), jnp.bfloat16),
            pltpu.VMEM((S, D), jnp.bfloat16),
            pltpu.VMEM((S, D), jnp.float32),
            pltpu.VMEM((NFC, D, FC), jnp.bfloat16),
            pltpu.VMEM((NFC, FC, D), jnp.bfloat16),
            pltpu.VMEM((WOFF + 98 * 512, 128), jnp.uint32),
            pltpu.VMEM((98, D // 2, DH), jnp.uint32),
            pltpu.VMEM((8, H * DH // 2, 128), jnp.uint32),
            pltpu.SemaphoreType.DMA((S // LB,)),
            pltpu.SemaphoreType.DMA((NFC,)),
            pltpu.SemaphoreType.DMA((NFC,)),
            pltpu.SemaphoreType.DMA((3,)),
            pltpu.SemaphoreType.DMA((1,)),
            pltpu.SemaphoreType.DMA((1,)),
        ],
        compiler_params=pltpu.CompilerParams(
            vmem_limit_bytes=120 * 1024 * 1024,
            flags={"XLA_TPU_RESCHEDULE_DMA_DONES": True},
        ),
    )(x, mem0, wq, wk, wv, wo, B_w1, b1, B_w2, b2)
    return out.reshape(1, S, D)
```

```python
import functools

import jax
import jax.numpy as jnp
from jax import lax
import jax.experimental.pallas as pl
import jax.experimental.pallas.tpu as pltpu

S, D, H, DH, M, SEG, F = 2048, 1024, 32, 128, 8, 32, 3584
L = M + SEG
NSEG = S // SEG
FC = 512
NFC = F // FC
RB = 1024
NRB = S // RB
NSUB = 8
SB = RB // NSUB
LB = 256
NEG = -1e9
BT, FT = 5, 11
UNR = 4
B2OFF = 256
WOFF = 512
CW = 2
NIT = (NFC - CW) * NRB
UPI = (48 + NIT - 1) // NIT
IT0 = CW * NRB
NPART = 4 * NSUB
H1 = 28


def _dot(a, b):
    return lax.dot_general(a, b, (((1,), (0,)), ((), ())), preferred_element_type=jnp.float32)


def _dot_nt(a, b):
    return lax.dot_general(a, b, (((1,), (1,)), ((), ())), preferred_element_type=jnp.float32)


def _kernel(x_hbm, mem0_hbm, wq_hbm, wk_hbm, wv_hbm, wo_hbm, w1_hbm, b1_hbm, w2_hbm, b2_hbm,
            o_hbm,
            x_s, xn_s, res_s, w1_s, w2_s, big_s, stage_s, wo_s, mem0_ref, b1_ref, b2_ref,
            sem_x, sem_w1, sem_w2, sem_st, sem_wo, sem_o, sem_small):
    def x_copy(r):
        r0 = pl.multiple_of(r * LB, LB)
        return pltpu.make_async_copy(x_hbm.at[pl.ds(r0, LB), :], x_s.at[pl.ds(r0, LB), :], sem_x.at[r])

    def w1_copy(c):
        c0 = pl.multiple_of(c * FC, FC)
        return pltpu.make_async_copy(w1_hbm.at[:, pl.ds(c0, FC)], w1_s.at[c], sem_w1.at[c])

    def w2_copy(c):
        c0 = pl.multiple_of(c * FC, FC)
        return pltpu.make_async_copy(w2_hbm.at[pl.ds(c0, FC), :], w2_s.at[c], sem_w2.at[c])

    def issue_x(lo, hi):
        def body(r, carry):
            x_copy(r).start()
            return carry
        lax.fori_loop(lo, hi, body, 0)

    def issue_w(lo, hi):
        def body(c, carry):
            w1_copy(c).start()
            w2_copy(c).start()
            return carry
        lax.fori_loop(lo, hi, body, 0)

    small = [pltpu.make_async_copy(b1_hbm, b1_ref, sem_small.at[0]),
             pltpu.make_async_copy(b2_hbm, b2_ref, sem_small.at[1]),
             pltpu.make_async_copy(mem0_hbm, mem0_ref, sem_small.at[2])]
    for cp in small:
        cp.start()
    issue_x(0, RB // LB)
    issue_w(0, 1)
    issue_x(RB // LB, S // LB)
    issue_w(1, NFC)

    c_st = [pltpu.make_async_copy(w.bitcast(jnp.uint32).at[:, i, :], stage_s.at[m * 32 + i], sem_st.at[m])
            for m, w in enumerate((wq_hbm, wk_hbm, wv_hbm)) for i in range(32)]
    c_wo = [pltpu.make_async_copy(wo_hbm.bitcast(jnp.uint32).at[:, pl.ds(n * 128, 128)], wo_s.at[n], sem_wo.at[0])
            for n in range(8)]
    late_copies = c_st + c_wo

    for cp in small:
        cp.wait()
    b1f = pltpu.bitcast(b1_ref[...].astype(jnp.float32), jnp.uint32)
    for i in range(F // 128):
        big_s[i * 8:(i + 1) * 8, :] = jnp.broadcast_to(b1f[i:i + 1, :], (8, 128))
    b2f = pltpu.bitcast(b2_ref[...].astype(jnp.float32), jnp.uint32)
    for n in range(D // 128):
        big_s[B2OFF + n * 8:B2OFF + (n + 1) * 8, :] = jnp.broadcast_to(b2f[n:n + 1, :], (8, 128))

    def ln_body(r, carry):
        x_copy(r).wait()
        r0 = pl.multiple_of(r * LB, LB)
        xb = x_s[pl.ds(r0, LB), :].astype(jnp.float32)
        mu = jnp.mean(xb, axis=-1, keepdims=True)
        xc = xb - mu
        var = jnp.mean(xc * xc, axis=-1, keepdims=True)
        xn = xc * lax.rsqrt(var + 1e-5)
        xn_s[pl.ds(r0, LB), :] = xn.astype(jnp.bfloat16)
        return carry

    def rp_part(p, it):
        tot = UPI * 64
        lo_, hi_ = (tot * p) // NPART, (tot * (p + 1)) // NPART
        for k in range(UPI):
            a0, a1 = max(lo_, k * 64) - k * 64, min(hi_, (k + 1) * 64) - k * 64
            if a1 <= a0:
                continue
            unit = (it - IT0) * UPI + k
            valid = jnp.logical_and(it >= IT0, unit < 48)
            m = unit // 16
            hp = unit % 16
            ei = jnp.where(valid, m * 32 + hp, 96)
            oi = jnp.where(valid, m * 32 + 16 + hp, 97)
            di = jnp.where(valid, m * 32 + 2 * hp, 96)
            e = stage_s[ei, a0 * 8:a1 * 8, :]
            o = stage_s[oi, a0 * 8:a1 * 8, :]
            lo = (e & jnp.uint32(0xFFFF)) | (o << 16)
            hi = (e >> 16) | (o & jnp.uint32(0xFFFF0000))
            d0 = pl.multiple_of(WOFF + di * 512 + a0 * 8, 8)
            big_s[pl.ds(d0, (a1 - a0) * 8), :] = lo
            big_s[pl.ds(d0 + 512, (a1 - a0) * 8), :] = hi

    def ffn_chunk(c, carry):
        for k in range(4):
            @pl.when(c == k)
            def _():
                for cp in late_copies[k * 32:(k + 1) * 32]:
                    cp.start()
        for m_ in range(3):
            first_it = IT0 + (16 * m_) // UPI
            assert first_it // NRB > m_

            @pl.when(c == first_it // NRB)
            def _():
                for cp in c_st[m_ * 32:(m_ + 1) * 32]:
                    cp.wait()

        def ffn_body(r, carry2):
            @pl.when(c == 0)
            def _():
                lax.fori_loop(r * (RB // LB), (r + 1) * (RB // LB), ln_body, 0)

            @pl.when(r == 0)
            def _():
                w1_copy(c).wait()
                w2_copy(c).wait()
            hc = {}

            def up(u):
                r0 = pl.multiple_of(r * RB + u * SB, SB)
                xb = xn_s[pl.ds(r0, SB), :]
                hs = []
                for i in range(FC // 128):
                    rp_part(u * 4 + i, c * NRB + r)
                    b0 = pl.multiple_of((c * 4 + i) * 8, 8)
                    b8 = pltpu.bitcast(big_s[pl.ds(b0, 8), :], jnp.float32)
                    a = _dot(xb, w1_s[c, :, i * 128:(i + 1) * 128]) + jnp.tile(b8, (SB // 8, 1))
                    g = jax.nn.gelu(a, approximate=True)
                    hs.append(g.astype(jnp.bfloat16))
                hc[u] = jnp.concatenate(hs, axis=1)

            def down(u):
                r0 = pl.multiple_of(r * RB + u * SB, SB)
                hcat = hc.pop(u)
                for n in range(D // 128):
                    y = _dot(hcat, w2_s[c, :, n * 128:(n + 1) * 128])
                    b8 = pltpu.bitcast(big_s[B2OFF + n * 8:B2OFF + (n + 1) * 8, :], jnp.float32)
                    prev = jnp.where(c == 0, jnp.tile(b8, (SB // 8, 1)),
                                     res_s[pl.ds(r0, SB), n * 128:(n + 1) * 128])
                    res_s[pl.ds(r0, SB), n * 128:(n + 1) * 128] = prev + y

            up(0)
            for u in range(NSUB):
                if u + 1 < NSUB:
                    up(u + 1)
                down(u)
            return carry2
        lax.fori_loop(0, NRB, ffn_body, 0)
        return carry
    lax.fori_loop(0, NFC, ffn_chunk, 0)
    for cp in c_wo:
        cp.wait()

    ri = lax.broadcasted_iota(jnp.int32, (L, 128), 0)
    ci = lax.broadcasted_iota(jnp.int32, (L, 128), 1)
    mask = ((ri < M) | (ri >= ci)) & (ci < L)
    scale = DH ** (-0.5)
    zpad = jnp.zeros((128 - L, DH), jnp.float32)

    def wrows(idx, a, b):
        return pltpu.bitcast(big_s[WOFF + idx * 512 + a:WOFF + idx * 512 + b, :], jnp.bfloat16)

    def out_copy(s):
        r0 = pl.multiple_of(s * SEG, SEG)
        return pltpu.make_async_copy(x_s.at[pl.ds(r0, SEG), :], o_hbm.at[pl.ds(r0, SEG), :], sem_o.at[0])

    def step(s, mem, maybe_first):
        if maybe_first:
            @pl.when(s > 0)
            def _():
                out_copy(s - 1).start()
        else:
            out_copy(s - 1).start()
        r0 = pl.multiple_of(s * SEG, SEG)
        xs = xn_s[pl.ds(r0, SEG), :].astype(jnp.float32)
        h = jnp.concatenate([mem, xs], axis=0)
        q_, k_, v_, p_, o_ = {}, {}, {}, {}, {}
        pre = {idx: _dot(h[:, :512], wrows(idx, 0, 256)) for idx in (0, 32, 64)}

        def proj(idx):
            if idx in pre:
                return _dot(h[:, 512:], wrows(idx, 256, 512)) + pre.pop(idx)
            return _dot(h, wrows(idx, 0, 512))

        def padded(t):
            return jnp.concatenate([t, zpad], axis=0).astype(jnp.bfloat16)

        def scores(j):
            sc = _dot_nt(q_.pop(j), k_.pop(j))
            t = jnp.where(mask, sc * scale, NEG)
            m = jnp.max(t, axis=1, keepdims=True)
            e = jnp.exp(t - m)
            l = jnp.sum(e, axis=1, keepdims=True)
            r_ = pl.reciprocal(l, approx=True)
            p_[j] = e * (r_ * (2.0 - l * r_))

        def values(j):
            o_[j] = _dot(p_.pop(j), v_.pop(j))

        def emit(t):
            if (t - BT) % 3 == 0 and 0 <= (t - BT) // 3 < H:
                scores((t - BT) // 3)
            if (t - FT) % 3 == 0 and 0 <= (t - FT) // 3 < H:
                values((t - FT) // 3)

        for i in range(H):
            q_[i] = proj(i)
            emit(3 * i)
            k_[i] = padded(proj(32 + i))
            emit(3 * i + 1)
            v_[i] = padded(proj(64 + i))
            emit(3 * i + 2)

        tail = sorted([(3 * j + BT, 0, j) for j in range(H) if 3 * j + BT >= 3 * H] +
                      [(3 * j + FT, 1, j) for j in range(H) if 3 * j + FT >= 3 * H])
        assert all(j >= H1 for _, _, j in tail)
        part1 = []

        def wo_part1(n):
            o1 = jnp.concatenate([o_[j] for j in range(H1)], axis=1)
            part1.append(_dot(o1, pltpu.bitcast(wo_s[n, 0:H1 * 64, :], jnp.bfloat16)))

        wo_part1(0)
        n_done = 1
        clock = 3 * H - 1 + 3.5
        for t, kind, j in tail:
            while clock < t and n_done < 8:
                wo_part1(n_done)
                n_done += 1
                clock += 3.5
            (scores if kind == 0 else values)(j)
        while n_done < 8:
            wo_part1(n_done)
            n_done += 1
        o2 = jnp.concatenate([o_[j] for j in range(H1, H)], axis=1)
        outs = [_dot(o2, pltpu.bitcast(wo_s[n, H1 * 64:H * 64, :], jnp.bfloat16)) + part1[n] for n in range(8)]
        out = jnp.concatenate(outs, axis=1)
        fin = (res_s[pl.ds(r0, SEG), :] + out[M:]) + x_s[pl.ds(r0, SEG), :].astype(jnp.float32)
        x_s[pl.ds(r0, SEG), :] = fin.astype(jnp.bfloat16)
        return out[:M]

    def steps(i, mem):
        for u in range(UNR):
            mem = step(i * UNR + u, mem, u == 0)
        return mem
    lax.fori_loop(0, NSEG // UNR, steps, mem0_ref[...].astype(jnp.float32))
    out_copy(NSEG - 1).start()
    pltpu.make_async_copy(x_s, o_hbm, sem_o.at[0]).wait()


@functools.partial(jax.jit, static_argnames=("A_seg_len",))
def pallas_parallel_sum__memory_aug_recurrent_mem_tr__dense_activation_gelu__prompt_kernel(
    A_x: jax.Array,
    A_mem0: jax.Array,
    A_Wq: jax.Array,
    A_Wk: jax.Array,
    A_Wv: jax.Array,
    A_Wo: jax.Array,
    A_seg_len: int,
    B_x: jax.Array,
    B_w1: jax.Array,
    B_b1: jax.Array,
    B_w2: jax.Array,
    B_b2: jax.Array,
):
    del B_x
    assert A_x.shape == (1, S, D) and A_mem0.shape == (1, M, D) and int(A_seg_len) == SEG
    assert A_Wq.shape == (D, H, DH) and A_Wo.shape == (H, DH, D) and B_w1.shape == (D, F)
    x = A_x.reshape(S, D)
    mem0 = A_mem0.reshape(M, D)
    wq = A_Wq.reshape(D // 2, 2 * H, DH)
    wk = A_Wk.reshape(D // 2, 2 * H, DH)
    wv = A_Wv.reshape(D // 2, 2 * H, DH)
    wo = A_Wo.reshape(H * DH, D)
    b1 = B_b1.reshape(F // 128, 128)
    b2 = B_b2.reshape(D // 128, 128)
    any_spec = pl.BlockSpec(memory_space=pl.ANY)
    out = pl.pallas_call(
        _kernel,
        out_shape=jax.ShapeDtypeStruct((S, D), jnp.bfloat16),
        in_specs=[any_spec] * 10,
        out_specs=any_spec,
        scratch_shapes=[
            pltpu.VMEM((S, D), jnp.bfloat16),
            pltpu.VMEM((S, D), jnp.bfloat16),
            pltpu.VMEM((S, D), jnp.float32),
            pltpu.VMEM((NFC, D, FC), jnp.bfloat16),
            pltpu.VMEM((NFC, FC, D), jnp.bfloat16),
            pltpu.VMEM((WOFF + 98 * 512, 128), jnp.uint32),
            pltpu.VMEM((98, D // 2, DH), jnp.uint32),
            pltpu.VMEM((8, H * DH // 2, 128), jnp.uint32),
            pltpu.VMEM((M, D), jnp.bfloat16),
            pltpu.VMEM((F // 128, 128), jnp.bfloat16),
            pltpu.VMEM((D // 128, 128), jnp.bfloat16),
            pltpu.SemaphoreType.DMA((S // LB,)),
            pltpu.SemaphoreType.DMA((NFC,)),
            pltpu.SemaphoreType.DMA((NFC,)),
            pltpu.SemaphoreType.DMA((3,)),
            pltpu.SemaphoreType.DMA((1,)),
            pltpu.SemaphoreType.DMA((1,)),
            pltpu.SemaphoreType.DMA((3,)),
        ],
        compiler_params=pltpu.CompilerParams(
            vmem_limit_bytes=120 * 1024 * 1024,
            flags={"XLA_TPU_RESCHEDULE_DMA_DONES": True},
        ),
    )(x, mem0, wq, wk, wv, wo, B_w1, b1, B_w2, b2)
    return out.reshape(1, S, D)
```

```python
import functools

import jax
import jax.numpy as jnp
from jax import lax
import jax.experimental.pallas as pl
import jax.experimental.pallas.tpu as pltpu

S, D, H, DH, M, SEG, F = 2048, 1024, 32, 128, 8, 32, 3584
L = M + SEG
NSEG = S // SEG
FC = 512
NFC = F // FC
RB = 1024
NRB = S // RB
NSUB = 8
SB = RB // NSUB
LB = 256
NEG = -1e9
BT, FT = 5, 11
UNR = 4
B2OFF = 256
WOFF = 512
CW = 2
NIT = (NFC - CW) * NRB
UPI = (48 + NIT - 1) // NIT
IT0 = CW * NRB
NPART = 4 * NSUB
H1 = 28


def _dot(a, b):
    return lax.dot_general(a, b, (((1,), (0,)), ((), ())), preferred_element_type=jnp.float32)


def _dot_nt(a, b):
    return lax.dot_general(a, b, (((1,), (1,)), ((), ())), preferred_element_type=jnp.float32)


def _kernel(x_hbm, mem0_hbm, wq_hbm, wk_hbm, wv_hbm, wo_hbm, w1_hbm, b1_hbm, w2_hbm, b2_hbm,
            o_hbm,
            x_s, xn_s, res_s, w1_s, w2_s, big_s, stage_s, wo_s, mem0_ref, b1_ref, b2_ref,
            sem_x, sem_w1, sem_w2, sem_st, sem_wo, sem_o, sem_small):
    def x_copy(r):
        r0 = pl.multiple_of(r * LB, LB)
        return pltpu.make_async_copy(x_hbm.at[pl.ds(r0, LB), :], x_s.at[pl.ds(r0, LB), :], sem_x.at[r])

    def w1_copy(c):
        c0 = pl.multiple_of(c * FC, FC)
        return pltpu.make_async_copy(w1_hbm.at[:, pl.ds(c0, FC)], w1_s.at[c], sem_w1.at[c])

    def w2_copy(c):
        c0 = pl.multiple_of(c * FC, FC)
        return pltpu.make_async_copy(w2_hbm.at[pl.ds(c0, FC), :], w2_s.at[c], sem_w2.at[c])

    def issue_x(lo, hi):
        def body(r, carry):
            x_copy(r).start()
            return carry
        lax.fori_loop(lo, hi, body, 0)

    def issue_w(lo, hi):
        def body(c, carry):
            w1_copy(c).start()
            w2_copy(c).start()
            return carry
        lax.fori_loop(lo, hi, body, 0)

    small = [pltpu.make_async_copy(b1_hbm, b1_ref, sem_small.at[0]),
             pltpu.make_async_copy(b2_hbm, b2_ref, sem_small.at[1]),
             pltpu.make_async_copy(mem0_hbm, mem0_ref, sem_small.at[2])]
    for cp in small:
        cp.start()
    issue_x(0, RB // LB)
    issue_w(0, 1)
    issue_x(RB // LB, S // LB)
    issue_w(1, NFC)

    c_st = [pltpu.make_async_copy(w.bitcast(jnp.uint32).at[:, i, :], stage_s.at[m * 32 + i], sem_st.at[m])
            for m, w in enumerate((wq_hbm, wk_hbm, wv_hbm)) for i in range(32)]
    c_wo = [pltpu.make_async_copy(wo_hbm.bitcast(jnp.uint32).at[:, pl.ds(n * 128, 128)], wo_s.at[n], sem_wo.at[0])
            for n in range(8)]
    late_copies = c_st + c_wo

    for cp in small:
        cp.wait()
    b1f = pltpu.bitcast(b1_ref[...].astype(jnp.float32), jnp.uint32)
    for i in range(F // 128):
        big_s[i * 8:(i + 1) * 8, :] = jnp.broadcast_to(b1f[i:i + 1, :], (8, 128))
    b2f = pltpu.bitcast(b2_ref[...].astype(jnp.float32), jnp.uint32)
    for n in range(D // 128):
        big_s[B2OFF + n * 8:B2OFF + (n + 1) * 8, :] = jnp.broadcast_to(b2f[n:n + 1, :], (8, 128))

    def ln_body(r, carry):
        x_copy(r).wait()
        r0 = pl.multiple_of(r * LB, LB)
        xb = x_s[pl.ds(r0, LB), :].astype(jnp.float32)
        mu = jnp.mean(xb, axis=-1, keepdims=True)
        xc = xb - mu
        var = jnp.mean(xc * xc, axis=-1, keepdims=True)
        xn = xc * lax.rsqrt(var + 1e-5)
        xn_s[pl.ds(r0, LB), :] = xn.astype(jnp.bfloat16)
        return carry

    def rp_part(p, it):
        tot = UPI * 64
        lo_, hi_ = (tot * p) // NPART, (tot * (p + 1)) // NPART
        for k in range(UPI):
            a0, a1 = max(lo_, k * 64) - k * 64, min(hi_, (k + 1) * 64) - k * 64
            if a1 <= a0:
                continue
            unit = (it - IT0) * UPI + k
            valid = jnp.logical_and(it >= IT0, unit < 48)
            m = unit // 16
            hp = unit % 16
            ei = jnp.where(valid, m * 32 + hp, 96)
            oi = jnp.where(valid, m * 32 + 16 + hp, 97)
            di = jnp.where(valid, m * 32 + 2 * hp, 96)
            e = stage_s[ei, a0 * 8:a1 * 8, :]
            o = stage_s[oi, a0 * 8:a1 * 8, :]
            lo = (e & jnp.uint32(0xFFFF)) | (o << 16)
            hi = (e >> 16) | (o & jnp.uint32(0xFFFF0000))
            d0 = pl.multiple_of(WOFF + di * 512 + a0 * 8, 8)
            big_s[pl.ds(d0, (a1 - a0) * 8), :] = lo
            big_s[pl.ds(d0 + 512, (a1 - a0) * 8), :] = hi

    def ffn_chunk(c, carry):
        for m_ in range(3):
            first_it = IT0 + (16 * m_) // UPI
            assert first_it // NRB > m_

            @pl.when(c == first_it // NRB)
            def _():
                for cp in c_st[m_ * 32:(m_ + 1) * 32]:
                    cp.wait()

        def ffn_body(r, carry2):
            @pl.when(c == 0)
            def _():
                lax.fori_loop(r * (RB // LB), (r + 1) * (RB // LB), ln_body, 0)

            @pl.when(r == 0)
            def _():
                w1_copy(c).wait()
                w2_copy(c).wait()
            hc = {}

            def up(u):
                for k in range(4):
                    cps = late_copies[k * 32:(k + 1) * 32]
                    for rr in range(NRB):
                        sel = cps[rr * len(cps) // NRB:(rr + 1) * len(cps) // NRB]
                        sel = sel[u * len(sel) // NSUB:(u + 1) * len(sel) // NSUB]
                        if sel:
                            @pl.when(jnp.logical_and(c == k, r == rr))
                            def _():
                                for cp in sel:
                                    cp.start()
                r0 = pl.multiple_of(r * RB + u * SB, SB)
                xb = xn_s[pl.ds(r0, SB), :]
                hs = []
                for i in range(FC // 128):
                    rp_part(u * 4 + i, c * NRB + r)
                    b0 = pl.multiple_of((c * 4 + i) * 8, 8)
                    b8 = pltpu.bitcast(big_s[pl.ds(b0, 8), :], jnp.float32)
                    a = _dot(xb, w1_s[c, :, i * 128:(i + 1) * 128]) + jnp.tile(b8, (SB // 8, 1))
                    g = jax.nn.gelu(a, approximate=True)
                    hs.append(g.astype(jnp.bfloat16))
                hc[u] = jnp.concatenate(hs, axis=1)

            def down(u):
                r0 = pl.multiple_of(r * RB + u * SB, SB)
                hcat = hc.pop(u)
                for n in range(D // 128):
                    y = _dot(hcat, w2_s[c, :, n * 128:(n + 1) * 128])
                    b8 = pltpu.bitcast(big_s[B2OFF + n * 8:B2OFF + (n + 1) * 8, :], jnp.float32)
                    prev = jnp.where(c == 0, jnp.tile(b8, (SB // 8, 1)),
                                     res_s[pl.ds(r0, SB), n * 128:(n + 1) * 128])
                    res_s[pl.ds(r0, SB), n * 128:(n + 1) * 128] = prev + y

            up(0)
            for u in range(NSUB):
                if u + 1 < NSUB:
                    up(u + 1)
                down(u)
            return carry2
        lax.fori_loop(0, NRB, ffn_body, 0)
        return carry
    lax.fori_loop(0, NFC, ffn_chunk, 0)
    for cp in c_wo:
        cp.wait()

    ri = lax.broadcasted_iota(jnp.int32, (L, 128), 0)
    ci = lax.broadcasted_iota(jnp.int32, (L, 128), 1)
    mask = ((ri < M) | (ri >= ci)) & (ci < L)
    scale = DH ** (-0.5)
    zpad = jnp.zeros((128 - L, DH), jnp.float32)

    def wrows(idx, a, b):
        return pltpu.bitcast(big_s[WOFF + idx * 512 + a:WOFF + idx * 512 + b, :], jnp.bfloat16)

    def out_copy(s):
        r0 = pl.multiple_of(s * SEG, SEG)
        return pltpu.make_async_copy(x_s.at[pl.ds(r0, SEG), :], o_hbm.at[pl.ds(r0, SEG), :], sem_o.at[0])

    def step(s, mem, maybe_first):
        if maybe_first:
            @pl.when(s > 0)
            def _():
                out_copy(s - 1).start()
        else:
            out_copy(s - 1).start()
        r0 = pl.multiple_of(s * SEG, SEG)
        xs = xn_s[pl.ds(r0, SEG), :].astype(jnp.float32)
        h = jnp.concatenate([mem, xs], axis=0)
        q_, k_, v_, p_, o_ = {}, {}, {}, {}, {}
        pre = {idx: _dot(h[:, :512], wrows(idx, 0, 256)) for idx in (0, 32, 64)}

        def proj(idx):
            if idx in pre:
                return _dot(h[:, 512:], wrows(idx, 256, 512)) + pre.pop(idx)
            return _dot(h, wrows(idx, 0, 512))

        def padded(t):
            return jnp.concatenate([t, zpad], axis=0).astype(jnp.bfloat16)

        def scores(j):
            sc = _dot_nt(q_.pop(j), k_.pop(j))
            t = jnp.where(mask, sc * scale, NEG)
            m = jnp.max(t, axis=1, keepdims=True)
            e = jnp.exp(t - m)
            l = jnp.sum(e, axis=1, keepdims=True)
            r_ = pl.reciprocal(l, approx=True)
            p_[j] = e * (r_ * (2.0 - l * r_))

        def values(j):
            o_[j] = _dot(p_.pop(j), v_.pop(j))

        def emit(t):
            if (t - BT) % 3 == 0 and 0 <= (t - BT) // 3 < H:
                scores((t - BT) // 3)
            if (t - FT) % 3 == 0 and 0 <= (t - FT) // 3 < H:
                values((t - FT) // 3)

        for i in range(H):
            q_[i] = proj(i)
            emit(3 * i)
            k_[i] = padded(proj(32 + i))
            emit(3 * i + 1)
            v_[i] = padded(proj(64 + i))
            emit(3 * i + 2)

        tail = sorted([(3 * j + BT, 0, j) for j in range(H) if 3 * j + BT >= 3 * H] +
                      [(3 * j + FT, 1, j) for j in range(H) if 3 * j + FT >= 3 * H])
        assert all(j >= H1 for _, _, j in tail)
        part1 = []

        def wo_part1(n):
            o1 = jnp.concatenate([o_[j] for j in range(H1)], axis=1)
            part1.append(_dot(o1, pltpu.bitcast(wo_s[n, 0:H1 * 64, :], jnp.bfloat16)))

        wo_part1(0)
        n_done = 1
        clock = 3 * H - 1 + 3.5
        for t, kind, j in tail:
            while clock < t and n_done < 8:
                wo_part1(n_done)
                n_done += 1
                clock += 3.5
            (scores if kind == 0 else values)(j)
        while n_done < 8:
            wo_part1(n_done)
            n_done += 1
        o2 = jnp.concatenate([o_[j] for j in range(H1, H)], axis=1)
        outs = [_dot(o2, pltpu.bitcast(wo_s[n, H1 * 64:H * 64, :], jnp.bfloat16)) + part1[n] for n in range(8)]
        out = jnp.concatenate(outs, axis=1)
        fin = (res_s[pl.ds(r0, SEG), :] + out[M:]) + x_s[pl.ds(r0, SEG), :].astype(jnp.float32)
        x_s[pl.ds(r0, SEG), :] = fin.astype(jnp.bfloat16)
        return out[:M]

    def steps(i, mem):
        for u in range(UNR):
            mem = step(i * UNR + u, mem, u == 0)
        return mem
    lax.fori_loop(0, NSEG // UNR, steps, mem0_ref[...].astype(jnp.float32))
    out_copy(NSEG - 1).start()
    pltpu.make_async_copy(x_s, o_hbm, sem_o.at[0]).wait()


@functools.partial(jax.jit, static_argnames=("A_seg_len",))
def pallas_parallel_sum__memory_aug_recurrent_mem_tr__dense_activation_gelu__prompt_kernel(
    A_x: jax.Array,
    A_mem0: jax.Array,
    A_Wq: jax.Array,
    A_Wk: jax.Array,
    A_Wv: jax.Array,
    A_Wo: jax.Array,
    A_seg_len: int,
    B_x: jax.Array,
    B_w1: jax.Array,
    B_b1: jax.Array,
    B_w2: jax.Array,
    B_b2: jax.Array,
):
    del B_x
    assert A_x.shape == (1, S, D) and A_mem0.shape == (1, M, D) and int(A_seg_len) == SEG
    assert A_Wq.shape == (D, H, DH) and A_Wo.shape == (H, DH, D) and B_w1.shape == (D, F)
    x = A_x.reshape(S, D)
    mem0 = A_mem0.reshape(M, D)
    wq = A_Wq.reshape(D // 2, 2 * H, DH)
    wk = A_Wk.reshape(D // 2, 2 * H, DH)
    wv = A_Wv.reshape(D // 2, 2 * H, DH)
    wo = A_Wo.reshape(H * DH, D)
    b1 = B_b1.reshape(F // 128, 128)
    b2 = B_b2.reshape(D // 128, 128)
    any_spec = pl.BlockSpec(memory_space=pl.ANY)
    out = pl.pallas_call(
        _kernel,
        out_shape=jax.ShapeDtypeStruct((S, D), jnp.bfloat16),
        in_specs=[any_spec] * 10,
        out_specs=any_spec,
        scratch_shapes=[
            pltpu.VMEM((S, D), jnp.bfloat16),
            pltpu.VMEM((S, D), jnp.bfloat16),
            pltpu.VMEM((S, D), jnp.float32),
            pltpu.VMEM((NFC, D, FC), jnp.bfloat16),
            pltpu.VMEM((NFC, FC, D), jnp.bfloat16),
            pltpu.VMEM((WOFF + 98 * 512, 128), jnp.uint32),
            pltpu.VMEM((98, D // 2, DH), jnp.uint32),
            pltpu.VMEM((8, H * DH // 2, 128), jnp.uint32),
            pltpu.VMEM((M, D), jnp.bfloat16),
            pltpu.VMEM((F // 128, 128), jnp.bfloat16),
            pltpu.VMEM((D // 128, 128), jnp.bfloat16),
            pltpu.SemaphoreType.DMA((S // LB,)),
            pltpu.SemaphoreType.DMA((NFC,)),
            pltpu.SemaphoreType.DMA((NFC,)),
            pltpu.SemaphoreType.DMA((3,)),
            pltpu.SemaphoreType.DMA((1,)),
            pltpu.SemaphoreType.DMA((1,)),
            pltpu.SemaphoreType.DMA((3,)),
        ],
        compiler_params=pltpu.CompilerParams(
            vmem_limit_bytes=120 * 1024 * 1024,
            flags={"XLA_TPU_RESCHEDULE_DMA_DONES": True},
        ),
    )(x, mem0, wq, wk, wv, wo, B_w1, b1, B_w2, b2)
    return out.reshape(1, S, D)
```
